```python
import jax
import jax.numpy as jnp

def _softmax(x, axis=-1):
    return jax.nn.softmax(x, axis=axis)
def _gelu(x):
    return jax.nn.gelu(x, approximate=True)
def _silu(x):
    return jax.nn.silu(x)
def _sigmoid(x):
    return jax.nn.sigmoid(x)
def _layernorm(x, axis=-1, eps=1e-5):
    m = jnp.mean(x, axis=axis, keepdims=True)
    v = jnp.var(x, axis=axis, keepdims=True)
    return (x - m) / jnp.sqrt(v + eps)
def _scatter_add(tgt, idx, src, axis=0):
    return tgt.at[idx].add(src)
def _segment_sum(src, seg, n):
    return jax.ops.segment_sum(src, seg, n)
class _Rng:
    def __init__(self, key):
        self._k = key
    def _next(self):
        self._k, sub = jax.random.split(self._k)
        return sub
    def normal(self, shape):
        return jax.random.normal(self._next(), shape, dtype=jnp.bfloat16)
    def randint(self, lo, hi, shape):
        return jax.random.randint(self._next(), shape, lo, hi, dtype=jnp.int32)
    def uniform(self, shape, lo=0.0, hi=1.0):
        return jax.random.uniform(self._next(), shape, jnp.bfloat16, lo, hi)
    def permutation(self, n):
        return jax.random.permutation(self._next(), n)


kernel_name = 'concat_heads__gqa_block_cached__compressed_kv_cla__decode'

def setup_inputs():
    _rng = _Rng(jax.random.key(int.from_bytes(__import__("os").urandom(4), "little")))
    _w = (lambda a: (lambda t: t.astype(jnp.bfloat16) if jnp.issubdtype(t.dtype, jnp.floating) else t)(jnp.asarray(a)))
    def _A_setup():
        B, Sq, D = 2, 1, 512
        Hq, Hkv, Sk, Dh = 32, 32, 8192, 128
        assert Hq % Hkv == 0, (Hq, Hkv)
        return {
            "x": _w((lambda *s: _rng.normal(s) * 0.05)(B, Sq, D)),
            "k_cache": _w((lambda *s: _rng.normal(s) * 0.05)(B, Hkv, Sk, Dh)),
            "v_cache": _w((lambda *s: _rng.normal(s) * 0.05)(B, Hkv, Sk, Dh)),
            "wq": _w((lambda *s: _rng.normal(s) * 0.05)(D, Hq * Dh) * (D ** -0.5)),
            "wo": _w((lambda *s: _rng.normal(s) * 0.05)(Hq * Dh, D) * ((Hq * Dh) ** -0.5)),
        }
    _A_in = _A_setup()

    def _B_setup():
        B, H, Sq, Sk, D, M = 2, 32, 1, 8192, 128, 512
        Dc = 4 * D
        return {
            "x": _w((lambda *s: _rng.normal(s) * 0.05)(B, Sq, M)),
            "c_kv": _w((lambda *s: _rng.normal(s) * 0.05)(B, Sk, Dc)),
            "w_q": _w((lambda *s: _rng.normal(s) * 0.05)(M, H, D) * (M ** -0.5)),
            "w_uk": _w((lambda *s: _rng.normal(s) * 0.05)(Dc, H, D) * (Dc ** -0.5)),
            "w_uv": _w((lambda *s: _rng.normal(s) * 0.05)(Dc, H, D) * (Dc ** -0.5)),
            "w_o": _w((lambda *s: _rng.normal(s) * 0.05)(H, D, M) * ((H * D) ** -0.5)),
        }
    _B_in = _B_setup()

    return {
        "A_x": _A_in["x"],
        "A_k_cache": _A_in["k_cache"],
        "A_v_cache": _A_in["v_cache"],
        "A_wq": _A_in["wq"],
        "A_wo": _A_in["wo"],
        "B_x": _B_in["x"],
        "B_c_kv": _B_in["c_kv"],
        "B_w_q": _B_in["w_q"],
        "B_w_uk": _B_in["w_uk"],
        "B_w_uv": _B_in["w_uv"],
        "B_w_o": _B_in["w_o"],
    }

def reference(A_x, A_k_cache, A_v_cache, A_wq, A_wo, B_x, B_c_kv, B_w_q, B_w_uk, B_w_uv, B_w_o):
    def _A_ref(x, k_cache, v_cache, wq, wo):
        B, Sq, D = x.shape
        Hq, Dh = 32, 128
        Hkv = k_cache.shape[1]
        rep = Hq // Hkv
        q = (lambda x, *d: x.transpose(*d))((x @ wq).reshape(B, Sq, Hq, Dh), 0, 2, 1, 3)
        k = jnp.repeat(k_cache, rep, axis=1)
        v = jnp.repeat(v_cache, rep, axis=1)
        scores = jnp.einsum("bhqd,bhkd->bhqk", q, k) * (Dh ** -0.5)
        p = _softmax(scores, axis=-1)
        o = jnp.einsum("bhqk,bhkd->bhqd", p, v)
        return (lambda x, *d: x.transpose(*d))(o, 0, 2, 1, 3).reshape(B, Sq, Hq * Dh) @ wo

    def _B_ref(x, c_kv, w_q, w_uk, w_uv, w_o):
        B, Sq, M = x.shape[0], x.shape[1], x.shape[2]
        Sk = c_kv.shape[1]
        H, D = w_q.shape[1], w_q.shape[2]
        q = jnp.einsum("bqm,mhd->bhqd", x, w_q)
        k = jnp.einsum("bkc,chd->bhkd", c_kv, w_uk)
        v = jnp.einsum("bkc,chd->bhkd", c_kv, w_uv)
        scores = jnp.einsum("bhqd,bhkd->bhqk", q, k) * (D ** -0.5)
        off = Sk - Sq
        qi = jnp.arange(Sq)[:, None]
        kj = jnp.arange(Sk)[None, :]
        cmask = kj <= (qi + off)
        scores = jnp.where(cmask[None, None], scores, -1e9)
        p = _softmax(scores, axis=-1)
        ctx = jnp.einsum("bhqk,bhkd->bhqd", p, v)
        return jnp.einsum("bhqd,hdm->bqm", ctx, w_o)

    a = _A_ref(A_x, A_k_cache, A_v_cache, A_wq, A_wo)
    b = _B_ref(B_x, B_c_kv, B_w_q, B_w_uk, B_w_uv, B_w_o)
    return jnp.concatenate([a, b], axis=-1)
```

```python
import jax
import jax.numpy as jnp
import jax.experimental.pallas as pl
import jax.experimental.pallas.tpu as pltpu

NB, NH, SK, DH, DM, DC = 2, 32, 8192, 128, 512, 512
NSLOT = 3
PIECE = 160
SCALE = DH ** -0.5
F32, BF16 = jnp.float32, jnp.bfloat16
NT = (((1,), (1,)), ((), ()))


def _kernel(xa_hbm, k_hbm, v_hbm, wq_hbm, wo_hbm, xb_hbm, ckv_hbm, wqb_hbm, wuk_hbm, wuv_hbm,
            wob_hbm, out_ref,
            xa_buf, xb_buf, wq_buf, wo_buf, wqb_buf, wuk_buf, wuv_buf, wob_buf, ckv_buf, kv_buf,
            qa_scr, qb_scr, qabs_scr, s_scr, ctx_scr, sems, kv_sems):
  cp = pltpu.make_async_copy

  def stream4(src, dst, sem, rows, piece, r0=0):
    q = rows // 4

    def body(j, c):
      for s in range(4):
        off = pl.multiple_of(r0 + s * q + j * piece, piece)
        cp(src.at[pl.ds(off, piece)], dst.at[pl.ds(off, piece)], sem).start(priority=s % 2)
      return c

    jax.lax.fori_loop(0, q // piece, body, 0)

  def stream_wq(sem):
    def body(j, c):
      r = pl.multiple_of(j * 16, 16)
      for s in range(4):
        cols = pl.ds(s * 1024, 1024)
        cp(wq_hbm.at[pl.ds(r, 16), cols], wq_buf.at[pl.ds(r, 16), cols], sem).start(priority=s % 2)
      return c

    jax.lax.fori_loop(0, DM // 16, body, 0)

  def wait_all(buf, sem):
    cp(buf, buf, sem).wait()

  n_full = SK // PIECE - (1 if SK % PIECE < PIECE // 2 else 0)
  last = SK - n_full * PIECE

  def start_kv(h, slot):
    def one(off, sz):
      for b in range(NB):
        cp(k_hbm.at[b, h, pl.ds(off, sz)], kv_buf.at[slot, 2 * b, pl.ds(off, sz)],
           kv_sems.at[slot, 0]).start(priority=0)
        cp(v_hbm.at[b, h, pl.ds(off, sz)], kv_buf.at[slot, 2 * b + 1, pl.ds(off, sz)],
           kv_sems.at[slot, 1]).start(priority=1)

    def body(j, c):
      one(pl.multiple_of(j * PIECE, 16), PIECE)
      return c

    jax.lax.fori_loop(0, n_full, body, 0)
    if last:
      one(n_full * PIECE, last)

  def wait_kv(slot):
    for i in range(2):
      for b in range(NB):
        wait_all(kv_buf.at[slot, 2 * b + i], kv_sems.at[slot, i])

  row8 = jax.lax.broadcasted_iota(jnp.int32, (8, 1), 0)
  is0 = row8 == 0

  def pad8(x_buf):
    x = x_buf[...].astype(F32)
    return jnp.concatenate([x, jnp.zeros((8 - NB, DM), F32)], axis=0).astype(BF16)

  def head_pair(w_buf, j):
    wu = w_buf.bitcast(jnp.uint32)[pl.ds(j, DM, stride=NH // 2), :]
    lo = pltpu.bitcast(wu << 16, F32).astype(BF16)
    hi = pltpu.bitcast(wu & jnp.uint32(0xFFFF0000), F32).astype(BF16)
    return lo, hi

  cp(xa_hbm, xa_buf, sems.at[0]).start()
  cp(xb_hbm, xb_buf, sems.at[1]).start()
  stream_wq(sems.at[2])
  stream4(wqb_hbm, wqb_buf, sems.at[3], DM * NH, 128)

  wait_all(xa_buf, sems.at[0])
  wait_all(wq_buf, sems.at[2])
  qa = jnp.dot(pad8(xa_buf), wq_buf[...], preferred_element_type=F32)
  for h in range(NH):
    qa_scr[h] = qa[:, h * DH:(h + 1) * DH]

  stream4(wuk_hbm, wuk_buf, sems.at[4], DC * NH, 128)
  wait_all(xb_buf, sems.at[1])
  wait_all(wqb_buf, sems.at[3])
  xb8 = pad8(xb_buf)

  def qb_body(j, c):
    lo, hi = head_pair(wqb_buf, j)
    qb_scr[2 * j] = jnp.dot(xb8, lo, preferred_element_type=F32)
    qb_scr[2 * j + 1] = jnp.dot(xb8, hi, preferred_element_type=F32)
    return c

  for j in range(NH // 2):
    qb_body(j, 0)

  HALF = SK // 2
  stream4(ckv_hbm.at[0], ckv_buf.at[0], sems.at[5], HALF, 32)
  wait_all(wuk_buf, sems.at[4])

  def qabs_body(j, c):
    ws = head_pair(wuk_buf, j)
    for e in range(2):
      h = 2 * j + e
      r = jax.lax.dot_general(qb_scr[h].astype(BF16), ws[e], NT, preferred_element_type=F32)
      for b in range(NB):
        qabs_scr[b, pl.ds(h, 1), :] = r[b:b + 1, :]
    return c

  for j in range(NH // 2):
    qabs_body(j, 0)

  CH = 1024

  def scores_b(b, half):
    qabs = qabs_scr[b].astype(BF16)

    def body(c, carry):
      r = pl.multiple_of(half * HALF + c * CH, CH)
      s = jax.lax.dot_general(qabs, ckv_buf[b, pl.ds(r, CH), :], NT, preferred_element_type=F32)
      s_scr[b, :, pl.ds(r, CH)] = s * SCALE
      return carry

    jax.lax.fori_loop(0, HALF // CH, body, 0)

  def softmax_pv_b(b):
    m = jnp.max(s_scr[b], axis=-1, keepdims=True)

    def body(c, carry):
      acc, l = carry
      r = pl.multiple_of(c * CH, CH)
      p = jnp.exp(s_scr[b, :, pl.ds(r, CH)] - m)
      l = l + jnp.sum(p, axis=-1, keepdims=True)
      acc = acc + jnp.dot(p.astype(BF16), ckv_buf[b, pl.ds(r, CH), :], preferred_element_type=F32)
      return acc, l

    acc, l = jax.lax.fori_loop(0, SK // CH, body,
                               (jnp.zeros((NH, DC), F32), jnp.zeros((NH, 1), F32)))
    ctx_scr[b] = acc / l

  stream4(ckv_hbm.at[0], ckv_buf.at[0], sems.at[6], HALF, 32, r0=HALF)
  wait_all(ckv_buf.at[0, pl.ds(0, HALF)], sems.at[5])
  scores_b(0, 0)
  stream4(ckv_hbm.at[1], ckv_buf.at[1], sems.at[7], HALF, 32)
  wait_all(ckv_buf.at[0, pl.ds(HALF, HALF)], sems.at[6])
  scores_b(0, 1)
  stream4(ckv_hbm.at[1], ckv_buf.at[1], sems.at[8], HALF, 32, r0=HALF)
  softmax_pv_b(0)
  stream4(wuv_hbm, wuv_buf, sems.at[9], DC * NH, 128)
  wait_all(ckv_buf.at[1, pl.ds(0, HALF)], sems.at[7])
  scores_b(1, 0)
  wait_all(ckv_buf.at[1, pl.ds(HALF, HALF)], sems.at[8])
  scores_b(1, 1)
  stream4(wob_hbm, wob_buf, sems.at[10], NH * DH, 32)
  softmax_pv_b(1)
  stream4(wo_hbm, wo_buf, sems.at[11], NH * DH, 32)
  start_kv(0, 0)
  wait_all(wuv_buf, sems.at[9])
  wait_all(wob_buf, sems.at[10])

  def outb_body(j, acc):
    ws = head_pair(wuv_buf, j)
    for e in range(2):
      h = 2 * j + e
      lhs = jnp.where(is0, ctx_scr[0, pl.ds(h, 1), :], ctx_scr[1, pl.ds(h, 1), :])
      ctx = jnp.dot(lhs.astype(BF16), ws[e], preferred_element_type=F32)
      acc = acc + jnp.dot(ctx.astype(BF16), wob_buf[pl.ds(pl.multiple_of(h * DH, DH), DH), :],
                          preferred_element_type=F32)
    return acc

  outb = jnp.zeros((8, DM), F32)
  for j in range(NH // 2):
    outb = outb_body(j, outb)
  out_ref[:, DM:2 * DM] = outb[0:NB].astype(BF16)

  for s in range(1, NSLOT - 1):
    start_kv(s, s)
  wait_all(wo_buf, sems.at[11])

  def head_body(h, acc):
    slot = h % NSLOT
    wait_kv(slot)
    q = qa_scr[h].astype(BF16)
    s0 = jax.lax.dot_general(q, kv_buf[slot, 0], NT, preferred_element_type=F32)
    s1 = jax.lax.dot_general(q, kv_buf[slot, 2], NT, preferred_element_type=F32)
    s = jnp.where(is0, s0, s1) * SCALE
    m = jnp.max(s, axis=-1, keepdims=True)
    p = jnp.exp(s - m)
    l = jnp.sum(p, axis=-1, keepdims=True)
    pb = p.astype(BF16)
    o0 = jnp.dot(pb, kv_buf[slot, 1], preferred_element_type=F32)
    o1 = jnp.dot(pb, kv_buf[slot, 3], preferred_element_type=F32)
    o = jnp.where(is0, o0, o1) / l
    acc = acc + jnp.dot(o.astype(BF16), wo_buf[pl.ds(pl.multiple_of(h * DH, DH), DH), :],
                        preferred_element_type=F32)

    nxt = h + NSLOT - 1

    @pl.when(nxt < NH)
    def _():
      start_kv(nxt, nxt % NSLOT)

    return acc

  outa = jax.lax.fori_loop(0, NH, head_body, jnp.zeros((8, DM), F32))
  out_ref[:, 0:DM] = outa[0:NB].astype(BF16)


@jax.jit
def pallas_concat_heads__gqa_block_cached__compressed_kv_cla__decode_kernel(
    A_x: jax.Array,
    A_k_cache: jax.Array,
    A_v_cache: jax.Array,
    A_wq: jax.Array,
    A_wo: jax.Array,
    B_x: jax.Array,
    B_c_kv: jax.Array,
    B_w_q: jax.Array,
    B_w_uk: jax.Array,
    B_w_uv: jax.Array,
    B_w_o: jax.Array,
):
  any_spec = pl.BlockSpec(memory_space=pl.ANY)
  vmem = pltpu.VMEM
  out = pl.pallas_call(
      _kernel,
      out_shape=jax.ShapeDtypeStruct((NB, 2 * DM), BF16),
      in_specs=[any_spec] * 11,
      out_specs=pl.BlockSpec(memory_space=vmem),
      scratch_shapes=[
          vmem((NB, DM), BF16), vmem((NB, DM), BF16),
          vmem((DM, NH * DH), BF16), vmem((NH * DH, DM), BF16),
          vmem((DM * NH, DH), BF16), vmem((DC * NH, DH), BF16), vmem((DC * NH, DH), BF16),
          vmem((NH * DH, DM), BF16),
          vmem((NB, SK, DC), BF16),
          vmem((NSLOT, 2 * NB, SK, DH), BF16),
          vmem((NH, 8, DH), F32), vmem((NH, 8, DH), F32),
          vmem((NB, NH, DC), F32), vmem((NB, NH, SK), F32), vmem((NB, NH, DC), F32),
          pltpu.SemaphoreType.DMA((12,)), pltpu.SemaphoreType.DMA((NSLOT, 2)),
      ],
      compiler_params=pltpu.CompilerParams(vmem_limit_bytes=100 * 1024 * 1024),
  )(
      A_x.reshape(NB, DM), A_k_cache, A_v_cache, A_wq, A_wo,
      B_x.reshape(NB, DM), B_c_kv,
      B_w_q.reshape(DM * NH, DH), B_w_uk.reshape(DC * NH, DH), B_w_uv.reshape(DC * NH, DH),
      B_w_o.reshape(NH * DH, DM),
  )
  return out.reshape(NB, 1, 2 * DM)
```

```python
import jax
import jax.numpy as jnp
import jax.experimental.pallas as pl
import jax.experimental.pallas.tpu as pltpu

NB, NH, SK, DH, DM, DC = 2, 32, 8192, 128, 512, 512
NSLOT = 3
PIECE = 160
WPIECE = 128
CPIECE = 32
WO_CH = 8
WO_EARLY = 7
CH = 1024
SCALE = DH ** -0.5
F32, BF16 = jnp.float32, jnp.bfloat16
NT = (((1,), (1,)), ((), ()))


def _kernel(xa_hbm, k_hbm, v_hbm, wq_hbm, wo_hbm, xb_hbm, ckv_hbm, wqb_hbm, wuk_hbm, wuv_hbm,
            wob_hbm, out_ref,
            xa_buf, xb_buf, wq_buf, wo_buf, wqb_buf, wuk_buf, wuv_buf, wob_buf, ckv_buf, kv_buf,
            qa_scr, qb_scr, qabs_scr, s_scr, ctx_scr, o_scr, sems, kv_sems, wo_sems):
  cp = pltpu.make_async_copy

  def stream4(src, dst, sem, rows, piece, r0=0):
    q = rows // 4
    assert q * 4 == rows and q % piece == 0

    def body(j, c):
      for s in range(4):
        off = pl.multiple_of(r0 + s * q + j * piece, piece)
        cp(src.at[pl.ds(off, piece)], dst.at[pl.ds(off, piece)], sem).start(priority=s % 2)
      return c

    jax.lax.fori_loop(0, q // piece, body, 0)

  def stream_wq(sem):
    def body(j, c):
      r = pl.multiple_of(j * 16, 16)
      for s in range(4):
        cols = pl.ds(s * 1024, 1024)
        cp(wq_hbm.at[pl.ds(r, 16), cols], wq_buf.at[pl.ds(r, 16), cols], sem).start(priority=s % 2)
      return c

    jax.lax.fori_loop(0, DM // 16, body, 0)

  def wait_all(buf, sem):
    cp(buf, buf, sem).wait()

  n_full = SK // PIECE - (1 if 0 < SK % PIECE < PIECE // 2 else 0)
  last = SK - n_full * PIECE

  def start_kv(h, slot, j0=0, j1=n_full):
    def one(off, sz):
      for b in range(NB):
        cp(k_hbm.at[b, h, pl.ds(off, sz)], kv_buf.at[slot, 2 * b, pl.ds(off, sz)],
           kv_sems.at[slot, 0]).start(priority=0)
        cp(v_hbm.at[b, h, pl.ds(off, sz)], kv_buf.at[slot, 2 * b + 1, pl.ds(off, sz)],
           kv_sems.at[slot, 1]).start(priority=1)

    def body(j, c):
      one(pl.multiple_of(j * PIECE, 16), PIECE)
      return c

    jax.lax.fori_loop(j0, j1, body, 0)
    if j1 == n_full and last:
      one(n_full * PIECE, last)

  def wait_kv(slot):
    for i in range(2):
      for b in range(NB):
        wait_all(kv_buf.at[slot, 2 * b + i], kv_sems.at[slot, i])

  WCR = NH * DH // WO_CH

  def start_wo(c0, c1):
    for c in range(c0, c1):
      stream4(wo_hbm, wo_buf, wo_sems.at[c], WCR, CPIECE, r0=c * WCR)

  is0 = jax.lax.broadcasted_iota(jnp.int32, (8, 1), 0) == 0

  def pad8(x_buf):
    x = x_buf[...].astype(F32)
    return jnp.concatenate([x, jnp.zeros((8 - NB, DM), F32)], axis=0).astype(BF16)

  def head_pair(w_buf, j):
    wu = w_buf.bitcast(jnp.uint32)[pl.ds(j, DM, stride=NH // 2), :]
    lo = pltpu.bitcast(wu << 16, F32).astype(BF16)
    hi = pltpu.bitcast(wu & jnp.uint32(0xFFFF0000), F32).astype(BF16)
    return lo, hi

  HALF = SK // 2

  def c_qa():
    qa = jnp.dot(pad8(xa_buf), wq_buf[...], preferred_element_type=F32)
    for h in range(NH):
      qa_scr[h] = qa[:, h * DH:(h + 1) * DH]

  def c_qb():
    xb8 = pad8(xb_buf)
    for j in range(NH // 2):
      lo, hi = head_pair(wqb_buf, j)
      qb_scr[2 * j] = jnp.dot(xb8, lo, preferred_element_type=F32)
      qb_scr[2 * j + 1] = jnp.dot(xb8, hi, preferred_element_type=F32)

  def c_qabs():
    for j in range(NH // 2):
      ws = head_pair(wuk_buf, j)
      for e in range(2):
        h = 2 * j + e
        r = jax.lax.dot_general(qb_scr[h].astype(BF16), ws[e], NT, preferred_element_type=F32)
        for b in range(NB):
          qabs_scr[b, pl.ds(h, 1), :] = r[b:b + 1, :]

  def c_scores(b, half):
    qabs = qabs_scr[b].astype(BF16)

    def body(c, carry):
      r = pl.multiple_of(half * HALF + c * CH, CH)
      s = jax.lax.dot_general(qabs, ckv_buf[b, pl.ds(r, CH), :], NT, preferred_element_type=F32)
      s_scr[b, :, pl.ds(r, CH)] = s * SCALE
      return carry

    jax.lax.fori_loop(0, HALF // CH, body, 0)

  def c_pv(b, half, m, carry):
    def body(c, carry):
      acc, l = carry
      r = pl.multiple_of(half * HALF + c * CH, CH)
      p = jnp.exp(s_scr[b, :, pl.ds(r, CH)] - m)
      l = l + jnp.sum(p, axis=-1, keepdims=True)
      acc = acc + jnp.dot(p.astype(BF16), ckv_buf[b, pl.ds(r, CH), :], preferred_element_type=F32)
      return acc, l

    return jax.lax.fori_loop(0, HALF // CH, body, carry)

  def c_outb(j0, j1, acc):
    for j in range(j0, j1):
      ws = head_pair(wuv_buf, j)
      for e in range(2):
        h = 2 * j + e
        lhs = jnp.where(is0, ctx_scr[0, pl.ds(h, 1), :], ctx_scr[1, pl.ds(h, 1), :])
        ctx = jnp.dot(lhs.astype(BF16), ws[e], preferred_element_type=F32)
        acc = acc + jnp.dot(ctx.astype(BF16), wob_buf[h * DH:(h + 1) * DH, :],
                            preferred_element_type=F32)
    return acc

  def c_head(h, slot):
    wait_kv(slot)
    q = qa_scr[h].astype(BF16)
    s0 = jax.lax.dot_general(q, kv_buf[slot, 0], NT, preferred_element_type=F32)
    s1 = jax.lax.dot_general(q, kv_buf[slot, 2], NT, preferred_element_type=F32)
    s = jnp.where(is0, s0, s1) * SCALE
    m = jnp.max(s, axis=-1, keepdims=True)
    p = jnp.exp(s - m)
    l = jnp.sum(p, axis=-1, keepdims=True)
    pb = p.astype(BF16)
    o0 = jnp.dot(pb, kv_buf[slot, 1], preferred_element_type=F32)
    o1 = jnp.dot(pb, kv_buf[slot, 3], preferred_element_type=F32)
    o_scr[h] = jnp.where(is0, o0, o1) / l

  def zero_carry():
    return jnp.zeros((NH, DC), F32), jnp.zeros((NH, 1), F32)

  cp(xa_hbm, xa_buf, sems.at[0]).start()
  cp(xb_hbm, xb_buf, sems.at[1]).start()
  stream_wq(sems.at[2])
  stream4(wqb_hbm, wqb_buf, sems.at[3], DM * NH, WPIECE)
  wait_all(xa_buf, sems.at[0])
  wait_all(wq_buf, sems.at[2])
  c_qa()
  stream4(wuk_hbm, wuk_buf, sems.at[4], DC * NH, WPIECE)
  wait_all(xb_buf, sems.at[1])
  wait_all(wqb_buf, sems.at[3])
  c_qb()
  stream4(ckv_hbm.at[0], ckv_buf.at[0], sems.at[5], HALF, CPIECE)
  wait_all(wuk_buf, sems.at[4])
  c_qabs()
  stream4(ckv_hbm.at[0], ckv_buf.at[0], sems.at[6], HALF, CPIECE, r0=HALF)
  wait_all(ckv_buf.at[0, pl.ds(0, HALF)], sems.at[5])
  c_scores(0, 0)
  stream4(ckv_hbm.at[1], ckv_buf.at[1], sems.at[7], HALF, CPIECE)
  wait_all(ckv_buf.at[0, pl.ds(HALF, HALF)], sems.at[6])
  c_scores(0, 1)
  stream4(ckv_hbm.at[1], ckv_buf.at[1], sems.at[8], HALF, CPIECE, r0=HALF)
  wait_all(ckv_buf.at[1, pl.ds(0, HALF)], sems.at[7])
  c_scores(1, 0)
  stream4(wuv_hbm, wuv_buf, sems.at[9], DC * NH, WPIECE)
  wait_all(ckv_buf.at[1, pl.ds(HALF, HALF)], sems.at[8])
  c_scores(1, 1)
  stream4(wob_hbm, wob_buf, sems.at[10], NH * DH, CPIECE)
  m0 = jnp.max(s_scr[0], axis=-1, keepdims=True)
  c0 = c_pv(0, 0, m0, zero_carry())
  t1, t2 = n_full // 3, 2 * n_full // 3
  start_kv(0, 0, 0, t1)
  c0 = c_pv(0, 1, m0, c0)
  ctx_scr[0] = c0[0] / c0[1]
  start_kv(0, 0, t1, t2)
  m1 = jnp.max(s_scr[1], axis=-1, keepdims=True)
  c1 = c_pv(1, 0, m1, zero_carry())
  start_kv(0, 0, t2, n_full)
  c1 = c_pv(1, 1, m1, c1)
  ctx_scr[1] = c1[0] / c1[1]
  start_kv(1, 1, 0, t1)
  wait_all(wuv_buf, sems.at[9])
  wait_all(wob_buf, sems.at[10])
  outb = c_outb(0, 6, jnp.zeros((8, DM), F32))
  start_kv(1, 1, t1, t2)
  outb = c_outb(6, 11, outb)
  start_kv(1, 1, t2, n_full)
  outb = c_outb(11, 16, outb)
  out_ref[:, DM:2 * DM] = outb[0:NB].astype(BF16)

  LOOK = NSLOT - 1
  for s in range(2, LOOK):
    start_kv(s, s)

  def head_body(h, c):
    c_head(h, h % NSLOT)
    start_kv(h + LOOK, (h + LOOK) % NSLOT)
    return c

  jax.lax.fori_loop(0, NH - LOOK, head_body, 0)

  prev = 0
  for i in range(LOOK):
    h = NH - LOOK + i
    c_head(h, h % NSLOT)
    nxt = WO_EARLY * (i + 1) // (LOOK - 1) if i < LOOK - 1 else WO_CH
    start_wo(prev, nxt)
    prev = nxt

  acc = jnp.zeros((8, DM), F32)
  hpc = NH // WO_CH
  for c in range(WO_CH):
    wait_all(wo_buf.at[pl.ds(c * WCR, WCR)], wo_sems.at[c])
    for h in range(c * hpc, (c + 1) * hpc):
      acc = acc + jnp.dot(o_scr[h].astype(BF16), wo_buf[h * DH:(h + 1) * DH, :],
                          preferred_element_type=F32)
  out_ref[:, 0:DM] = acc[0:NB].astype(BF16)


@jax.jit
def pallas_concat_heads__gqa_block_cached__compressed_kv_cla__decode_kernel(
    A_x: jax.Array,
    A_k_cache: jax.Array,
    A_v_cache: jax.Array,
    A_wq: jax.Array,
    A_wo: jax.Array,
    B_x: jax.Array,
    B_c_kv: jax.Array,
    B_w_q: jax.Array,
    B_w_uk: jax.Array,
    B_w_uv: jax.Array,
    B_w_o: jax.Array,
):
  any_spec = pl.BlockSpec(memory_space=pl.ANY)
  vmem = pltpu.VMEM
  out = pl.pallas_call(
      _kernel,
      out_shape=jax.ShapeDtypeStruct((NB, 2 * DM), BF16),
      in_specs=[any_spec] * 11,
      out_specs=pl.BlockSpec(memory_space=vmem),
      scratch_shapes=[
          vmem((NB, DM), BF16), vmem((NB, DM), BF16),
          vmem((DM, NH * DH), BF16), vmem((NH * DH, DM), BF16),
          vmem((DM * NH, DH), BF16), vmem((DC * NH, DH), BF16), vmem((DC * NH, DH), BF16),
          vmem((NH * DH, DM), BF16),
          vmem((NB, SK, DC), BF16),
          vmem((NSLOT, 2 * NB, SK, DH), BF16),
          vmem((NH, 8, DH), F32), vmem((NH, 8, DH), F32),
          vmem((NB, NH, DC), F32), vmem((NB, NH, SK), F32), vmem((NB, NH, DC), F32),
          vmem((NH, 8, DH), F32),
          pltpu.SemaphoreType.DMA((11,)), pltpu.SemaphoreType.DMA((NSLOT, 2)),
          pltpu.SemaphoreType.DMA((WO_CH,)),
      ],
      compiler_params=pltpu.CompilerParams(vmem_limit_bytes=100 * 1024 * 1024),
  )(
      A_x.reshape(NB, DM), A_k_cache, A_v_cache, A_wq, A_wo,
      B_x.reshape(NB, DM), B_c_kv,
      B_w_q.reshape(DM * NH, DH), B_w_uk.reshape(DC * NH, DH), B_w_uv.reshape(DC * NH, DH),
      B_w_o.reshape(NH * DH, DM),
  )
  return out.reshape(NB, 1, 2 * DM)
```

```python
import jax
import jax.numpy as jnp
import jax.experimental.pallas as pl
import jax.experimental.pallas.tpu as pltpu

NB, NH, SK, DH, DM, DC = 2, 32, 8192, 128, 512, 512
NSLOT = 4
PARTS = 2
PIECE = 160
WPIECE = 128
CPIECE = 32
WO_CH = 8
WO_EARLY = 7
CH = 1024
SCALE = DH ** -0.5
F32, BF16 = jnp.float32, jnp.bfloat16
NT = (((1,), (1,)), ((), ()))


def _kernel(xa_hbm, k_hbm, v_hbm, wq_hbm, wo_hbm, xb_hbm, ckv_hbm, wqb_hbm, wuk_hbm, wuv_hbm,
            wob_hbm, out_ref,
            xa_buf, xb_buf, wq_buf, wo_buf, wqb_buf, wuk_buf, wuv_buf, wob_buf, ckv_buf, kv_buf,
            qa_scr, qb_scr, qabs_scr, s_scr, ctx_scr, o_scr, sems, kv_sems, wo_sems):
  cp = pltpu.make_async_copy

  def stream4(src, dst, sem, rows, piece, r0=0):
    q = rows // 4
    assert q * 4 == rows and q % piece == 0

    def body(j, c):
      for s in range(4):
        off = pl.multiple_of(r0 + s * q + j * piece, piece)
        cp(src.at[pl.ds(off, piece)], dst.at[pl.ds(off, piece)], sem).start(priority=s % 2)
      return c

    jax.lax.fori_loop(0, q // piece, body, 0)

  def stream_wq(sem):
    def body(j, c):
      r = pl.multiple_of(j * 16, 16)
      for s in range(4):
        cols = pl.ds(s * 1024, 1024)
        cp(wq_hbm.at[pl.ds(r, 16), cols], wq_buf.at[pl.ds(r, 16), cols], sem).start(priority=s % 2)
      return c

    jax.lax.fori_loop(0, DM // 16, body, 0)

  def wait_all(buf, sem):
    cp(buf, buf, sem).wait()

  PR = SK // PARTS
  n_full = PR // PIECE - (1 if 0 < PR % PIECE < PIECE // 2 else 0)
  last = PR - n_full * PIECE

  def start_kv(h, slot, j0=0, j1=n_full):
    def one(off, sz):
      for part in range(PARTS):
        rows = pl.ds(pl.multiple_of(off + part * PR, 16), sz)
        for b in range(NB):
          cp(k_hbm.at[b, h, rows], kv_buf.at[slot, 0, b, rows],
             kv_sems.at[slot, 0]).start(priority=0)
          cp(v_hbm.at[b, h, rows], kv_buf.at[slot, 1, b, rows],
             kv_sems.at[slot, 1]).start(priority=1)

    def body(j, c):
      one(j * PIECE, PIECE)
      return c

    jax.lax.fori_loop(j0, j1, body, 0)
    if j1 == n_full and last:
      one(n_full * PIECE, last)

  def wait_kv(slot):
    for i in range(2):
      wait_all(kv_buf.at[slot, i], kv_sems.at[slot, i])

  WCR = NH * DH // WO_CH

  def start_wo(c0, c1):
    for c in range(c0, c1):
      stream4(wo_hbm, wo_buf, wo_sems.at[c], WCR, CPIECE, r0=c * WCR)

  is0 = jax.lax.broadcasted_iota(jnp.int32, (8, 1), 0) == 0

  def pad8(x_buf):
    x = x_buf[...].astype(F32)
    return jnp.concatenate([x, jnp.zeros((8 - NB, DM), F32)], axis=0).astype(BF16)

  def head_pair(w_buf, j):
    wu = w_buf.bitcast(jnp.uint32)[pl.ds(j, DM, stride=NH // 2), :]
    lo = pltpu.bitcast(wu << 16, F32).astype(BF16)
    hi = pltpu.bitcast(wu & jnp.uint32(0xFFFF0000), F32).astype(BF16)
    return lo, hi

  HALF = SK // 2

  def c_qa():
    qa = jnp.dot(pad8(xa_buf), wq_buf[...], preferred_element_type=F32)
    for h in range(NH):
      qa_scr[h] = qa[:, h * DH:(h + 1) * DH]

  def c_qb():
    xb8 = pad8(xb_buf)
    for j in range(NH // 2):
      lo, hi = head_pair(wqb_buf, j)
      qb_scr[2 * j] = jnp.dot(xb8, lo, preferred_element_type=F32)
      qb_scr[2 * j + 1] = jnp.dot(xb8, hi, preferred_element_type=F32)

  def c_qabs():
    for j in range(NH // 2):
      ws = head_pair(wuk_buf, j)
      for e in range(2):
        h = 2 * j + e
        r = jax.lax.dot_general(qb_scr[h].astype(BF16), ws[e], NT, preferred_element_type=F32)
        for b in range(NB):
          qabs_scr[b, pl.ds(h, 1), :] = r[b:b + 1, :]

  def c_scores(b, half):
    qabs = qabs_scr[b].astype(BF16)

    def body(c, carry):
      r = pl.multiple_of(half * HALF + c * CH, CH)
      s = jax.lax.dot_general(qabs, ckv_buf[b, pl.ds(r, CH), :], NT, preferred_element_type=F32)
      s_scr[b, :, pl.ds(r, CH)] = s * SCALE
      return carry

    jax.lax.fori_loop(0, HALF // CH, body, 0)

  def c_pv(b, half, m, carry):
    def body(c, carry):
      acc, l = carry
      r = pl.multiple_of(half * HALF + c * CH, CH)
      p = jnp.exp(s_scr[b, :, pl.ds(r, CH)] - m)
      l = l + jnp.sum(p, axis=-1, keepdims=True)
      acc = acc + jnp.dot(p.astype(BF16), ckv_buf[b, pl.ds(r, CH), :], preferred_element_type=F32)
      return acc, l

    return jax.lax.fori_loop(0, HALF // CH, body, carry)

  def c_outb(j0, j1, acc):
    for j in range(j0, j1):
      ws = head_pair(wuv_buf, j)
      for e in range(2):
        h = 2 * j + e
        lhs = jnp.where(is0, ctx_scr[0, pl.ds(h, 1), :], ctx_scr[1, pl.ds(h, 1), :])
        ctx = jnp.dot(lhs.astype(BF16), ws[e], preferred_element_type=F32)
        acc = acc + jnp.dot(ctx.astype(BF16), wob_buf[h * DH:(h + 1) * DH, :],
                            preferred_element_type=F32)
    return acc

  def c_head(h, slot):
    wait_kv(slot)
    q = qa_scr[h].astype(BF16)
    s0 = jax.lax.dot_general(q, kv_buf[slot, 0, 0], NT, preferred_element_type=F32)
    s1 = jax.lax.dot_general(q, kv_buf[slot, 0, 1], NT, preferred_element_type=F32)
    s = jnp.where(is0, s0, s1) * SCALE
    m = jnp.max(s, axis=-1, keepdims=True)
    p = jnp.exp(s - m)
    l = jnp.sum(p, axis=-1, keepdims=True)
    pb = p.astype(BF16)
    o0 = jnp.dot(pb, kv_buf[slot, 1, 0], preferred_element_type=F32)
    o1 = jnp.dot(pb, kv_buf[slot, 1, 1], preferred_element_type=F32)
    o_scr[h] = jnp.where(is0, o0, o1) / l

  def zero_carry():
    return jnp.zeros((NH, DC), F32), jnp.zeros((NH, 1), F32)

  cp(xa_hbm, xa_buf, sems.at[0]).start()
  cp(xb_hbm, xb_buf, sems.at[1]).start()
  stream_wq(sems.at[2])
  stream4(wqb_hbm, wqb_buf, sems.at[3], DM * NH, WPIECE)
  wait_all(xa_buf, sems.at[0])
  wait_all(wq_buf, sems.at[2])
  c_qa()
  stream4(wuk_hbm, wuk_buf, sems.at[4], DC * NH, WPIECE)
  wait_all(xb_buf, sems.at[1])
  wait_all(wqb_buf, sems.at[3])
  c_qb()
  stream4(ckv_hbm.at[0], ckv_buf.at[0], sems.at[5], HALF, CPIECE)
  wait_all(wuk_buf, sems.at[4])
  c_qabs()
  stream4(ckv_hbm.at[0], ckv_buf.at[0], sems.at[6], HALF, CPIECE, r0=HALF)
  wait_all(ckv_buf.at[0, pl.ds(0, HALF)], sems.at[5])
  c_scores(0, 0)
  stream4(ckv_hbm.at[1], ckv_buf.at[1], sems.at[7], HALF, CPIECE)
  wait_all(ckv_buf.at[0, pl.ds(HALF, HALF)], sems.at[6])
  c_scores(0, 1)
  stream4(ckv_hbm.at[1], ckv_buf.at[1], sems.at[8], HALF, CPIECE, r0=HALF)
  wait_all(ckv_buf.at[1, pl.ds(0, HALF)], sems.at[7])
  c_scores(1, 0)
  stream4(wuv_hbm, wuv_buf, sems.at[9], DC * NH, WPIECE)
  wait_all(ckv_buf.at[1, pl.ds(HALF, HALF)], sems.at[8])
  c_scores(1, 1)
  stream4(wob_hbm, wob_buf, sems.at[10], NH * DH, CPIECE)
  m0 = jnp.max(s_scr[0], axis=-1, keepdims=True)
  c0 = c_pv(0, 0, m0, zero_carry())
  t1, t2 = n_full // 3, 2 * n_full // 3
  start_kv(0, 0, 0, t1)
  c0 = c_pv(0, 1, m0, c0)
  ctx_scr[0] = c0[0] / c0[1]
  start_kv(0, 0, t1, t2)
  m1 = jnp.max(s_scr[1], axis=-1, keepdims=True)
  c1 = c_pv(1, 0, m1, zero_carry())
  start_kv(0, 0, t2, n_full)
  c1 = c_pv(1, 1, m1, c1)
  ctx_scr[1] = c1[0] / c1[1]
  start_kv(1, 1, 0, t1)
  wait_all(wuv_buf, sems.at[9])
  wait_all(wob_buf, sems.at[10])
  outb = c_outb(0, 6, jnp.zeros((8, DM), F32))
  start_kv(1, 1, t1, t2)
  outb = c_outb(6, 11, outb)
  start_kv(1, 1, t2, n_full)
  outb = c_outb(11, 16, outb)
  out_ref[:, DM:2 * DM] = outb[0:NB].astype(BF16)

  LOOK = NSLOT - 1
  for s in range(2, LOOK):
    start_kv(s, s)

  def head_body(h, c):
    c_head(h, h % NSLOT)
    start_kv(h + LOOK, (h + LOOK) % NSLOT)
    return c

  jax.lax.fori_loop(0, NH - LOOK, head_body, 0)

  prev = 0
  for i in range(LOOK):
    h = NH - LOOK + i
    c_head(h, h % NSLOT)
    nxt = WO_EARLY * (i + 1) // (LOOK - 1) if i < LOOK - 1 else WO_CH
    start_wo(prev, nxt)
    prev = nxt

  acc = jnp.zeros((8, DM), F32)
  hpc = NH // WO_CH
  for c in range(WO_CH):
    wait_all(wo_buf.at[pl.ds(c * WCR, WCR)], wo_sems.at[c])
    for h in range(c * hpc, (c + 1) * hpc):
      acc = acc + jnp.dot(o_scr[h].astype(BF16), wo_buf[h * DH:(h + 1) * DH, :],
                          preferred_element_type=F32)
  out_ref[:, 0:DM] = acc[0:NB].astype(BF16)


@jax.jit
def pallas_concat_heads__gqa_block_cached__compressed_kv_cla__decode_kernel(
    A_x: jax.Array,
    A_k_cache: jax.Array,
    A_v_cache: jax.Array,
    A_wq: jax.Array,
    A_wo: jax.Array,
    B_x: jax.Array,
    B_c_kv: jax.Array,
    B_w_q: jax.Array,
    B_w_uk: jax.Array,
    B_w_uv: jax.Array,
    B_w_o: jax.Array,
):
  any_spec = pl.BlockSpec(memory_space=pl.ANY)
  vmem = pltpu.VMEM
  out = pl.pallas_call(
      _kernel,
      out_shape=jax.ShapeDtypeStruct((NB, 2 * DM), BF16),
      in_specs=[any_spec] * 11,
      out_specs=pl.BlockSpec(memory_space=vmem),
      scratch_shapes=[
          vmem((NB, DM), BF16), vmem((NB, DM), BF16),
          vmem((DM, NH * DH), BF16), vmem((NH * DH, DM), BF16),
          vmem((DM * NH, DH), BF16), vmem((DC * NH, DH), BF16), vmem((DC * NH, DH), BF16),
          vmem((NH * DH, DM), BF16),
          vmem((NB, SK, DC), BF16),
          vmem((NSLOT, 2, NB, SK, DH), BF16),
          vmem((NH, 8, DH), F32), vmem((NH, 8, DH), F32),
          vmem((NB, NH, DC), F32), vmem((NB, NH, SK), F32), vmem((NB, NH, DC), F32),
          vmem((NH, 8, DH), F32),
          pltpu.SemaphoreType.DMA((11,)), pltpu.SemaphoreType.DMA((NSLOT, 2)),
          pltpu.SemaphoreType.DMA((WO_CH,)),
      ],
      compiler_params=pltpu.CompilerParams(vmem_limit_bytes=100 * 1024 * 1024),
  )(
      A_x.reshape(NB, DM), A_k_cache, A_v_cache, A_wq, A_wo,
      B_x.reshape(NB, DM), B_c_kv,
      B_w_q.reshape(DM * NH, DH), B_w_uk.reshape(DC * NH, DH), B_w_uv.reshape(DC * NH, DH),
      B_w_o.reshape(NH * DH, DM),
  )
  return out.reshape(NB, 1, 2 * DM)
```

```python
import jax
import jax.numpy as jnp
import jax.experimental.pallas as pl
import jax.experimental.pallas.tpu as pltpu

NB, NH, SK, DH, DM, DC = 2, 32, 8192, 128, 512, 512
NSLOT = 4
PARTS = 2
PIECE = 160
WPIECE = 4
CPIECE = 32
WO_CH = 8
WO_EARLY = 7
CH = 1024
LEAD = 2
SCALE = DH ** -0.5
F32, BF16 = jnp.float32, jnp.bfloat16
NT = (((1,), (1,)), ((), ()))


def _kernel(xa_hbm, k_hbm, v_hbm, wq_hbm, wo_hbm, xb_hbm, ckv_hbm, wqb_hbm, wuk_hbm, wuv_hbm,
            wob_hbm, out_ref,
            xa_buf, xb_buf, wq_buf, wo_buf, wqb_buf, wuk_buf, wuv_buf, wob_buf, ckv_buf, kv_buf,
            qa_scr, qb_scr, qabs_scr, s_scr, ctx_scr, o_scr, sems, kv_sems, wo_sems):
  cp = pltpu.make_async_copy

  def stream4(src, dst, sem, rows, piece, r0=0, half=None):
    q = rows // 4
    assert q * 4 == rows and q % piece == 0
    n = q // piece
    j0, j1 = (0, n) if half is None else (half * n // 2, (half + 1) * n // 2)

    def body(j, c):
      for s in range(4):
        off = pl.multiple_of(r0 + s * q + j * piece, piece)
        cp(src.at[pl.ds(off, piece)], dst.at[pl.ds(off, piece)], sem).start(priority=s % 2)
      return c

    jax.lax.fori_loop(j0, j1, body, 0)

  def stream_wq(half):
    def body(j, c):
      rows = pl.ds(pl.multiple_of(j * 16, 16), 16)
      for s in range(4):
        cols = pl.ds(s * 1024, 1024)
        cp(wq_hbm.at[rows, cols], wq_buf.at[rows, cols], sems.at[2]).start(priority=s % 2)
      return c

    jax.lax.fori_loop(half * DM // 32, (half + 1) * DM // 32, body, 0)

  def wait_all(buf, sem):
    cp(buf, buf, sem).wait()

  PR = SK // PARTS
  n_full = PR // PIECE - (1 if 0 < PR % PIECE < PIECE // 2 else 0)
  last = PR - n_full * PIECE

  def start_kv(h, slot, j0=0, j1=n_full):
    def one(off, sz):
      for part in range(PARTS):
        rows = pl.ds(pl.multiple_of(off + part * PR, 16), sz)
        for b in range(NB):
          cp(k_hbm.at[b, h, rows], kv_buf.at[slot, 0, b, rows],
             kv_sems.at[slot, 0]).start(priority=0)
          cp(v_hbm.at[b, h, rows], kv_buf.at[slot, 1, b, rows],
             kv_sems.at[slot, 1]).start(priority=1)

    def body(j, c):
      one(j * PIECE, PIECE)
      return c

    jax.lax.fori_loop(j0, j1, body, 0)
    if j1 == n_full and last:
      one(n_full * PIECE, last)

  WCR = NH * DH // WO_CH

  def start_wo(c0, c1):
    for c in range(c0, c1):
      stream4(wo_hbm, wo_buf, wo_sems.at[c], WCR, CPIECE, r0=c * WCR)

  is0 = jax.lax.broadcasted_iota(jnp.int32, (8, 1), 0) == 0

  def pad8(x_buf):
    x = x_buf[...].astype(F32)
    return jnp.concatenate([x, jnp.zeros((8 - NB, DM), F32)], axis=0).astype(BF16)

  HALF = SK // 2

  def c_qa():
    qa = jnp.dot(pad8(xa_buf), wq_buf[...], preferred_element_type=F32)
    for h in range(NH):
      qa_scr[h] = qa[:, h * DH:(h + 1) * DH]

  def c_qb(h0, h1):
    xb8 = pad8(xb_buf)
    for h in range(h0, h1):
      qb_scr[h] = jnp.dot(xb8, wqb_buf[:, h, :], preferred_element_type=F32)

  def c_qabs(h0, h1):
    for h in range(h0, h1):
      r = jax.lax.dot_general(qb_scr[h].astype(BF16), wuk_buf[:, h, :], NT,
                              preferred_element_type=F32)
      for b in range(NB):
        qabs_scr[b, pl.ds(h, 1), :] = r[b:b + 1, :]

  def c_scores(b, half):
    qabs = qabs_scr[b].astype(BF16)

    def body(c, carry):
      r = pl.multiple_of(half * HALF + c * CH, CH)
      s = jax.lax.dot_general(qabs, ckv_buf[b, pl.ds(r, CH), :], NT, preferred_element_type=F32)
      s_scr[b, :, pl.ds(r, CH)] = s * SCALE
      return carry

    jax.lax.fori_loop(0, HALF // CH, body, 0)

  def c_pv(b, half, m, carry):
    def body(c, carry):
      acc, l = carry
      r = pl.multiple_of(half * HALF + c * CH, CH)
      p = jnp.exp(s_scr[b, :, pl.ds(r, CH)] - m)
      l = l + jnp.sum(p, axis=-1, keepdims=True)
      acc = acc + jnp.dot(p.astype(BF16), ckv_buf[b, pl.ds(r, CH), :], preferred_element_type=F32)
      return acc, l

    return jax.lax.fori_loop(0, HALF // CH, body, carry)

  def c_outb(h0, h1, acc):
    for h in range(h0, h1):
      lhs = jnp.where(is0, ctx_scr[0, pl.ds(h, 1), :], ctx_scr[1, pl.ds(h, 1), :])
      ctx = jnp.dot(lhs.astype(BF16), wuv_buf[:, h, :], preferred_element_type=F32)
      acc = acc + jnp.dot(ctx.astype(BF16), wob_buf[h * DH:(h + 1) * DH, :],
                          preferred_element_type=F32)
    return acc

  def c_head(h, slot):
    for i in range(2):
      wait_all(kv_buf.at[slot, i], kv_sems.at[slot, i])
    q = qa_scr[h].astype(BF16)
    s0 = jax.lax.dot_general(q, kv_buf[slot, 0, 0], NT, preferred_element_type=F32)
    s1 = jax.lax.dot_general(q, kv_buf[slot, 0, 1], NT, preferred_element_type=F32)
    s = jnp.where(is0, s0, s1) * SCALE
    m = jnp.max(s, axis=-1, keepdims=True)
    p = jnp.exp(s - m)
    l = jnp.sum(p, axis=-1, keepdims=True)
    pb = p.astype(BF16)
    o0 = jnp.dot(pb, kv_buf[slot, 1, 0], preferred_element_type=F32)
    o1 = jnp.dot(pb, kv_buf[slot, 1, 1], preferred_element_type=F32)
    o_scr[h] = jnp.where(is0, o0, o1) / l

  def zero_carry():
    return jnp.zeros((NH, DC), F32), jnp.zeros((NH, 1), F32)

  def split(n):
    return [(NH * i // n, NH * (i + 1) // n) for i in range(n)]

  LOOK = NSLOT - 1
  thirds = [0, n_full // 3, 2 * n_full // 3, n_full]

  def first_unit():
    cp(xa_hbm, xa_buf, sems.at[0]).start()
    cp(xb_hbm, xb_buf, sems.at[1]).start()
    stream_wq(0)

  units = [first_unit, lambda: stream_wq(1)]
  for src, dst, i in ((wqb_hbm, wqb_buf, 3), (wuk_hbm, wuk_buf, 4)):
    for half in range(2):
      units.append(lambda src=src, dst=dst, i=i, half=half:
                   stream4(src, dst, sems.at[i], DM, WPIECE, half=half))
  for b in range(NB):
    for hf in range(2):
      for half in range(2):
        units.append(lambda b=b, hf=hf, half=half: stream4(
            ckv_hbm.at[b], ckv_buf.at[b], sems.at[5 + 2 * b + hf], HALF, CPIECE,
            r0=hf * HALF, half=half))
  for half in range(2):
    units.append(lambda half=half: stream4(wuv_hbm, wuv_buf, sems.at[9], DC, WPIECE, half=half))
  for half in range(2):
    units.append(lambda half=half:
                 stream4(wob_hbm, wob_buf, sems.at[10], NH * DH, CPIECE, half=half))
  for h in range(LOOK):
    for t in range(3):
      units.append(lambda h=h, t=t: start_kv(h, h, thirds[t], thirds[t + 1]))

  issued = [0]

  def enqueue_upto(n):
    while issued[0] < min(n, len(units)):
      units[issued[0]]()
      issued[0] += 1

  def enqueue_one():
    enqueue_upto(issued[0] + 1)

  enqueue_upto(2 + LEAD)
  wait_all(xa_buf, sems.at[0])
  wait_all(wq_buf, sems.at[2])
  c_qa()
  enqueue_one()
  enqueue_upto(4 + LEAD)
  wait_all(xb_buf, sems.at[1])
  wait_all(wqb_buf, sems.at[3])
  for h0, h1 in split(4):
    c_qb(h0, h1)
    enqueue_one()
  enqueue_upto(6 + LEAD)
  wait_all(wuk_buf, sems.at[4])
  for h0, h1 in split(4):
    c_qabs(h0, h1)
    enqueue_one()
  for b in range(NB):
    for hf in range(2):
      enqueue_upto(8 + 2 * (2 * b + hf) + LEAD)
      wait_all(ckv_buf.at[b, pl.ds(hf * HALF, HALF)], sems.at[5 + 2 * b + hf])
      c_scores(b, hf)
      enqueue_one()
  for b in range(NB):
    m = jnp.max(s_scr[b], axis=-1, keepdims=True)
    carry = zero_carry()
    for hf in range(2):
      carry = c_pv(b, hf, m, carry)
      if hf == 1:
        ctx_scr[b] = carry[0] / carry[1]
      enqueue_one()
  enqueue_upto(18 + LEAD)
  wait_all(wuv_buf, sems.at[9])
  wait_all(wob_buf, sems.at[10])
  outb = jnp.zeros((8, DM), F32)
  for h0, h1 in split(5):
    outb = c_outb(h0, h1, outb)
    enqueue_one()
  out_ref[:, DM:2 * DM] = outb[0:NB].astype(BF16)
  enqueue_upto(len(units))

  def head_body(h, c):
    c_head(h, h % NSLOT)
    start_kv(h + LOOK, (h + LOOK) % NSLOT)
    return c

  jax.lax.fori_loop(0, NH - LOOK, head_body, 0)

  prev = 0
  for i in range(LOOK):
    h = NH - LOOK + i
    c_head(h, h % NSLOT)
    nxt = WO_EARLY * (i + 1) // (LOOK - 1) if i < LOOK - 1 else WO_CH
    start_wo(prev, nxt)
    prev = nxt

  acc = jnp.zeros((8, DM), F32)
  hpc = NH // WO_CH
  for c in range(WO_CH):
    wait_all(wo_buf.at[pl.ds(c * WCR, WCR)], wo_sems.at[c])
    for h in range(c * hpc, (c + 1) * hpc):
      acc = acc + jnp.dot(o_scr[h].astype(BF16), wo_buf[h * DH:(h + 1) * DH, :],
                          preferred_element_type=F32)
  out_ref[:, 0:DM] = acc[0:NB].astype(BF16)


@jax.jit
def pallas_concat_heads__gqa_block_cached__compressed_kv_cla__decode_kernel(
    A_x: jax.Array,
    A_k_cache: jax.Array,
    A_v_cache: jax.Array,
    A_wq: jax.Array,
    A_wo: jax.Array,
    B_x: jax.Array,
    B_c_kv: jax.Array,
    B_w_q: jax.Array,
    B_w_uk: jax.Array,
    B_w_uv: jax.Array,
    B_w_o: jax.Array,
):
  any_spec = pl.BlockSpec(memory_space=pl.ANY)
  vmem = pltpu.VMEM
  out = pl.pallas_call(
      _kernel,
      out_shape=jax.ShapeDtypeStruct((NB, 2 * DM), BF16),
      in_specs=[any_spec] * 11,
      out_specs=pl.BlockSpec(memory_space=vmem),
      scratch_shapes=[
          vmem((NB, DM), BF16), vmem((NB, DM), BF16),
          vmem((DM, NH * DH), BF16), vmem((NH * DH, DM), BF16),
          vmem((DM, NH, DH), BF16), vmem((DC, NH, DH), BF16), vmem((DC, NH, DH), BF16),
          vmem((NH * DH, DM), BF16),
          vmem((NB, SK, DC), BF16),
          vmem((NSLOT, 2, NB, SK, DH), BF16),
          vmem((NH, 8, DH), F32), vmem((NH, 8, DH), F32),
          vmem((NB, NH, DC), F32), vmem((NB, NH, SK), F32), vmem((NB, NH, DC), F32),
          vmem((NH, 8, DH), F32),
          pltpu.SemaphoreType.DMA((11,)), pltpu.SemaphoreType.DMA((NSLOT, 2)),
          pltpu.SemaphoreType.DMA((WO_CH,)),
      ],
      compiler_params=pltpu.CompilerParams(vmem_limit_bytes=100 * 1024 * 1024),
  )(
      A_x.reshape(NB, DM), A_k_cache, A_v_cache, A_wq, A_wo,
      B_x.reshape(NB, DM), B_c_kv, B_w_q, B_w_uk, B_w_uv, B_w_o.reshape(NH * DH, DM),
  )
  return out.reshape(NB, 1, 2 * DM)
```

```python
import jax
import jax.numpy as jnp
import jax.experimental.pallas as pl
import jax.experimental.pallas.tpu as pltpu

NB, NH, SK, DH, DM, DC = 2, 32, 8192, 128, 512, 512
NSLOT = 4
PARTS = 2
PIECE = 80
WPIECE = 4
CPIECE = 32
WO_CH = 8
WO_EARLY = 7
CH = 1024
LEAD = 2
SCALE = DH ** -0.5
F32, BF16 = jnp.float32, jnp.bfloat16
NT = (((1,), (1,)), ((), ()))


def _kernel(xa_hbm, k_hbm, v_hbm, wq_hbm, wo_hbm, xb_hbm, ckv_hbm, wqb_hbm, wuk_hbm, wuv_hbm,
            wob_hbm, out_ref,
            xa_buf, xb_buf, wq_buf, wo_buf, wqb_buf, wuk_buf, wuv_buf, wob_buf, ckv_buf, kv_buf,
            qa_scr, qb_scr, qabs_scr, s_scr, ctx_scr, o_scr, sems, kv_sems, wo_sems):
  cp = pltpu.make_async_copy

  def stream4(src, dst, sem, rows, piece, r0=0, half=None):
    q = rows // 4
    assert q * 4 == rows and q % piece == 0
    n = q // piece
    j0, j1 = (0, n) if half is None else (half * n // 2, (half + 1) * n // 2)

    def body(j, c):
      for s in range(4):
        off = pl.multiple_of(r0 + s * q + j * piece, piece)
        cp(src.at[pl.ds(off, piece)], dst.at[pl.ds(off, piece)], sem).start(priority=s % 2)
      return c

    jax.lax.fori_loop(j0, j1, body, 0)

  def stream_wq(half):
    def body(j, c):
      rows = pl.ds(pl.multiple_of(j * 16, 16), 16)
      for s in range(4):
        cols = pl.ds(s * 1024, 1024)
        cp(wq_hbm.at[rows, cols], wq_buf.at[rows, cols], sems.at[2]).start(priority=s % 2)
      return c

    jax.lax.fori_loop(half * DM // 32, (half + 1) * DM // 32, body, 0)

  def wait_all(buf, sem):
    cp(buf, buf, sem).wait()

  PR = SK // PARTS
  n_full = PR // PIECE - (1 if 0 < PR % PIECE < PIECE // 2 else 0)
  last = PR - n_full * PIECE
  assert PIECE % 16 == 0 and last % 16 == 0

  def start_kv(h, slot, j0=0, j1=n_full):
    def one(off, sz):
      rows = pl.ds(pl.multiple_of(off, 16), sz)
      for b in range(NB):
        cp(k_hbm.at[b, h, :, rows], kv_buf.at[slot, 0, b, :, rows],
           kv_sems.at[slot, 0]).start(priority=0)
        cp(v_hbm.at[b, h, :, rows], kv_buf.at[slot, 1, b, :, rows],
           kv_sems.at[slot, 1]).start(priority=1)

    def body(j, c):
      one(j * PIECE, PIECE)
      return c

    jax.lax.fori_loop(j0, j1, body, 0)
    if j1 == n_full and last:
      one(n_full * PIECE, last)

  WCR = NH * DH // WO_CH

  def start_wo(c0, c1):
    for c in range(c0, c1):
      stream4(wo_hbm, wo_buf, wo_sems.at[c], WCR, CPIECE, r0=c * WCR)

  is0 = jax.lax.broadcasted_iota(jnp.int32, (8, 1), 0) == 0

  def pad8(x_buf):
    x = x_buf[...].astype(F32)
    return jnp.concatenate([x, jnp.zeros((8 - NB, DM), F32)], axis=0).astype(BF16)

  HALF = SK // 2

  def c_qa():
    qa = jnp.dot(pad8(xa_buf), wq_buf[...], preferred_element_type=F32)
    for h in range(NH):
      qa_scr[h] = qa[:, h * DH:(h + 1) * DH]

  def c_qb(h0, h1):
    xb8 = pad8(xb_buf)
    for h in range(h0, h1):
      qb_scr[h] = jnp.dot(xb8, wqb_buf[:, h, :], preferred_element_type=F32)

  def c_qabs(h0, h1):
    for h in range(h0, h1):
      r = jax.lax.dot_general(qb_scr[h].astype(BF16), wuk_buf[:, h, :], NT,
                              preferred_element_type=F32)
      for b in range(NB):
        qabs_scr[b, pl.ds(h, 1), :] = r[b:b + 1, :]

  def c_scores(b, half):
    qabs = qabs_scr[b].astype(BF16)

    def body(c, carry):
      r = pl.multiple_of(half * HALF + c * CH, CH)
      s = jax.lax.dot_general(qabs, ckv_buf[b, pl.ds(r, CH), :], NT, preferred_element_type=F32)
      s_scr[b, :, pl.ds(r, CH)] = s * SCALE
      return carry

    jax.lax.fori_loop(0, HALF // CH, body, 0)

  def c_pv(b, half, m, carry):
    def body(c, carry):
      acc, l = carry
      r = pl.multiple_of(half * HALF + c * CH, CH)
      p = jnp.exp(s_scr[b, :, pl.ds(r, CH)] - m)
      l = l + jnp.sum(p, axis=-1, keepdims=True)
      acc = acc + jnp.dot(p.astype(BF16), ckv_buf[b, pl.ds(r, CH), :], preferred_element_type=F32)
      return acc, l

    return jax.lax.fori_loop(0, HALF // CH, body, carry)

  def c_outb(h0, h1, acc):
    for h in range(h0, h1):
      lhs = jnp.where(is0, ctx_scr[0, pl.ds(h, 1), :], ctx_scr[1, pl.ds(h, 1), :])
      ctx = jnp.dot(lhs.astype(BF16), wuv_buf[:, h, :], preferred_element_type=F32)
      acc = acc + jnp.dot(ctx.astype(BF16), wob_buf[h * DH:(h + 1) * DH, :],
                          preferred_element_type=F32)
    return acc

  def c_head(h, slot):
    for i in range(2):
      wait_all(kv_buf.at[slot, i], kv_sems.at[slot, i])
    q = qa_scr[h].astype(BF16)
    slab = lambda i, b: kv_buf[slot, i, b].reshape(SK, DH)
    s0 = jax.lax.dot_general(q, slab(0, 0), NT, preferred_element_type=F32)
    s1 = jax.lax.dot_general(q, slab(0, 1), NT, preferred_element_type=F32)
    s = jnp.where(is0, s0, s1) * SCALE
    m = jnp.max(s, axis=-1, keepdims=True)
    p = jnp.exp(s - m)
    l = jnp.sum(p, axis=-1, keepdims=True)
    pb = p.astype(BF16)
    o0 = jnp.dot(pb, slab(1, 0), preferred_element_type=F32)
    o1 = jnp.dot(pb, slab(1, 1), preferred_element_type=F32)
    o_scr[h] = jnp.where(is0, o0, o1) / l

  def zero_carry():
    return jnp.zeros((NH, DC), F32), jnp.zeros((NH, 1), F32)

  def split(n):
    return [(NH * i // n, NH * (i + 1) // n) for i in range(n)]

  LOOK = NSLOT - 1
  thirds = [0, n_full // 3, 2 * n_full // 3, n_full]

  def first_unit():
    cp(xa_hbm, xa_buf, sems.at[0]).start()
    cp(xb_hbm, xb_buf, sems.at[1]).start()
    stream_wq(0)

  units = [first_unit, lambda: stream_wq(1)]
  for src, dst, i in ((wqb_hbm, wqb_buf, 3), (wuk_hbm, wuk_buf, 4)):
    for half in range(2):
      units.append(lambda src=src, dst=dst, i=i, half=half:
                   stream4(src, dst, sems.at[i], DM, WPIECE, half=half))
  for b in range(NB):
    for hf in range(2):
      for half in range(2):
        units.append(lambda b=b, hf=hf, half=half: stream4(
            ckv_hbm.at[b], ckv_buf.at[b], sems.at[5 + 2 * b + hf], HALF, CPIECE,
            r0=hf * HALF, half=half))
  for half in range(2):
    units.append(lambda half=half: stream4(wuv_hbm, wuv_buf, sems.at[9], DC, WPIECE, half=half))
  for half in range(2):
    units.append(lambda half=half:
                 stream4(wob_hbm, wob_buf, sems.at[10], NH * DH, CPIECE, half=half))
  for h in range(LOOK):
    for t in range(3):
      units.append(lambda h=h, t=t: start_kv(h, h, thirds[t], thirds[t + 1]))

  issued = [0]

  def enqueue_upto(n):
    while issued[0] < min(n, len(units)):
      units[issued[0]]()
      issued[0] += 1

  def enqueue_one():
    enqueue_upto(issued[0] + 1)

  enqueue_upto(2 + LEAD)
  wait_all(xa_buf, sems.at[0])
  wait_all(wq_buf, sems.at[2])
  c_qa()
  enqueue_one()
  enqueue_upto(4 + LEAD)
  wait_all(xb_buf, sems.at[1])
  wait_all(wqb_buf, sems.at[3])
  for h0, h1 in split(4):
    c_qb(h0, h1)
    enqueue_one()
  enqueue_upto(6 + LEAD)
  wait_all(wuk_buf, sems.at[4])
  for h0, h1 in split(4):
    c_qabs(h0, h1)
    enqueue_one()
  for b in range(NB):
    for hf in range(2):
      enqueue_upto(8 + 2 * (2 * b + hf) + LEAD)
      wait_all(ckv_buf.at[b, pl.ds(hf * HALF, HALF)], sems.at[5 + 2 * b + hf])
      c_scores(b, hf)
      enqueue_one()
  for b in range(NB):
    m = jnp.max(s_scr[b], axis=-1, keepdims=True)
    carry = zero_carry()
    for hf in range(2):
      carry = c_pv(b, hf, m, carry)
      if hf == 1:
        ctx_scr[b] = carry[0] / carry[1]
      enqueue_one()
  enqueue_upto(18 + LEAD)
  wait_all(wuv_buf, sems.at[9])
  wait_all(wob_buf, sems.at[10])
  outb = jnp.zeros((8, DM), F32)
  for h0, h1 in split(5):
    outb = c_outb(h0, h1, outb)
    enqueue_one()
  out_ref[:, DM:2 * DM] = outb[0:NB].astype(BF16)
  enqueue_upto(len(units))

  def head_body(h, c):
    c_head(h, h % NSLOT)
    start_kv(h + LOOK, (h + LOOK) % NSLOT)
    return c

  jax.lax.fori_loop(0, NH - LOOK, head_body, 0)

  prev = 0
  for i in range(LOOK):
    h = NH - LOOK + i
    c_head(h, h % NSLOT)
    nxt = WO_EARLY * (i + 1) // (LOOK - 1) if i < LOOK - 1 else WO_CH
    start_wo(prev, nxt)
    prev = nxt

  acc = jnp.zeros((8, DM), F32)
  hpc = NH // WO_CH
  for c in range(WO_CH):
    wait_all(wo_buf.at[pl.ds(c * WCR, WCR)], wo_sems.at[c])
    for h in range(c * hpc, (c + 1) * hpc):
      acc = acc + jnp.dot(o_scr[h].astype(BF16), wo_buf[h * DH:(h + 1) * DH, :],
                          preferred_element_type=F32)
  out_ref[:, 0:DM] = acc[0:NB].astype(BF16)


@jax.jit
def pallas_concat_heads__gqa_block_cached__compressed_kv_cla__decode_kernel(
    A_x: jax.Array,
    A_k_cache: jax.Array,
    A_v_cache: jax.Array,
    A_wq: jax.Array,
    A_wo: jax.Array,
    B_x: jax.Array,
    B_c_kv: jax.Array,
    B_w_q: jax.Array,
    B_w_uk: jax.Array,
    B_w_uv: jax.Array,
    B_w_o: jax.Array,
):
  any_spec = pl.BlockSpec(memory_space=pl.ANY)
  vmem = pltpu.VMEM
  out = pl.pallas_call(
      _kernel,
      out_shape=jax.ShapeDtypeStruct((NB, 2 * DM), BF16),
      in_specs=[any_spec] * 11,
      out_specs=pl.BlockSpec(memory_space=vmem),
      scratch_shapes=[
          vmem((NB, DM), BF16), vmem((NB, DM), BF16),
          vmem((DM, NH * DH), BF16), vmem((NH * DH, DM), BF16),
          vmem((DM, NH, DH), BF16), vmem((DC, NH, DH), BF16), vmem((DC, NH, DH), BF16),
          vmem((NH * DH, DM), BF16),
          vmem((NB, SK, DC), BF16),
          vmem((NSLOT, 2, NB, PARTS, SK // PARTS, DH), BF16),
          vmem((NH, 8, DH), F32), vmem((NH, 8, DH), F32),
          vmem((NB, NH, DC), F32), vmem((NB, NH, SK), F32), vmem((NB, NH, DC), F32),
          vmem((NH, 8, DH), F32),
          pltpu.SemaphoreType.DMA((11,)), pltpu.SemaphoreType.DMA((NSLOT, 2)),
          pltpu.SemaphoreType.DMA((WO_CH,)),
      ],
      compiler_params=pltpu.CompilerParams(vmem_limit_bytes=100 * 1024 * 1024),
  )(
      A_x.reshape(NB, DM),
      A_k_cache.reshape(NB, NH, PARTS, SK // PARTS, DH),
      A_v_cache.reshape(NB, NH, PARTS, SK // PARTS, DH),
      A_wq, A_wo,
      B_x.reshape(NB, DM), B_c_kv, B_w_q, B_w_uk, B_w_uv, B_w_o.reshape(NH * DH, DM),
  )
  return out.reshape(NB, 1, 2 * DM)
```
